```python
import os as _os
_os.environ.setdefault("JAX_PLATFORMS", "cpu")
import jax
import jax.numpy as jnp

def _softmax(x, axis=-1):
    return jax.nn.softmax(x, axis=axis)
def _gelu(x):
    return jax.nn.gelu(x, approximate=True)
def _silu(x):
    return jax.nn.silu(x)
def _sigmoid(x):
    return jax.nn.sigmoid(x)
def _layernorm(x, axis=-1, eps=1e-5):
    m = jnp.mean(x, axis=axis, keepdims=True)
    v = jnp.var(x, axis=axis, keepdims=True)
    return (x - m) / jnp.sqrt(v + eps)
def _scatter_add(tgt, idx, src, axis=0):
    return tgt.at[idx].add(src)
def _segment_sum(src, seg, n):
    return jax.ops.segment_sum(src, seg, n)
class _Rng:
    def __init__(self, key):
        self._k = key
    def _next(self):
        self._k, sub = jax.random.split(self._k)
        return sub
    def normal(self, shape):
        return jax.random.normal(self._next(), shape, dtype=jnp.bfloat16)
    def randint(self, lo, hi, shape):
        return jax.random.randint(self._next(), shape, lo, hi, dtype=jnp.int32)
    def uniform(self, shape, lo=0.0, hi=1.0):
        return jax.random.uniform(self._next(), shape, jnp.bfloat16, lo, hi)
    def permutation(self, n):
        return jax.random.permutation(self._next(), n)


kernel_name = 'standalone__moe_arch_mod__prompt'

def setup_inputs():
    _rng = _Rng(jax.random.key(int.from_bytes(__import__("os").urandom(4), "little")))
    _w = (lambda a: (lambda t: t.astype(jnp.bfloat16) if jnp.issubdtype(t.dtype, jnp.floating) else t)(jnp.asarray(a)))
    B, S, D, F, C = 1, 2048, 576, 4608, 8
    return {
        "x": _w((lambda *s: _rng.normal(s) * 0.1)(B, S, D)),
        "w_r": _w((lambda *s: _rng.normal(s) * 0.1)(D)),
        "w_gate": _w((lambda *s: _rng.normal(s) * 0.1)(D, F)),
        "w_up": _w((lambda *s: _rng.normal(s) * 0.1)(D, F)),
        "w_down": _w((lambda *s: _rng.normal(s) * 0.1)(F, D)),
    }

def reference(x, w_r, w_gate, w_up, w_down):
    B, S, D = x.shape
    C = 8
    r = x @ w_r
    idx = jnp.argsort(-r, axis=-1)[:, :C]
    idx_e = jnp.repeat(idx.reshape(B, C, 1), D, axis=2)
    x_sel = jnp.take_along_axis(x, idx_e, axis=1)
    g = _silu(x_sel @ w_gate)
    u = x_sel @ w_up
    y = (g * u) @ w_down
    r_sel = _sigmoid(jnp.take_along_axis(r, idx, axis=1))
    y = y * r_sel.reshape(B, C, 1)
    b_off = (jnp.arange(B) * S).reshape(B, 1)
    flat_idx = (idx + b_off).reshape(B * C)
    zero = (x * 0.0).reshape(B * S, D)
    upd = _scatter_add(zero, flat_idx, y.reshape(B * C, D), axis=0)
    return x + upd.reshape(B, S, D)
```

```python
import jax
import jax.numpy as jnp
from jax import lax
import jax.experimental.pallas as pl
import jax.experimental.pallas.tpu as pltpu

_CAPACITY = 8
_GROUPS = 4
_TILE = 8
_F_CHUNK = 512
_UP_ROWS = (384, 576)
_EARLY_ROWS = (32, 64, 96)
_MID_ROWS = 128
_TRAILING_BANDS = 1


def _mod_kernel(x_hbm, wr_hbm, wg_hbm, wu_hbm, wd_hbm, o_hbm,
                x_v, wr_v, wg_v, wu_v, wd_v, o_v, g_v, h_v, out_sem):
    bands, rows, S = x_hbm.shape
    D, F = wg_hbm.shape
    C = _CAPACITY
    f32, bf16 = jnp.float32, jnp.bfloat16

    def start_writes(lo, hi):
        for r in range(lo, hi, _TILE):
            idx = (slice(None), pl.ds(r, _TILE))
            pltpu.make_async_copy(o_v.at[idx], o_hbm.at[idx], out_sem).start()

    def read_and_compute(sems):
        def copy(src, dst, sem, idx=None):
            if idx is not None:
                src, dst = src.at[idx], dst.at[idx]
            return pltpu.make_async_copy(src, dst, sems.at[sem])

        up_spans = list(zip((0,) + _UP_ROWS[:-1], _UP_ROWS))
        early_spans = list(zip((0,) + _EARLY_ROWS[:-1], _EARLY_ROWS))
        early_end = _EARLY_ROWS[-1]

        router_in = [copy(x_hbm, x_v, 0), copy(wr_hbm, wr_v, 0)]
        gate_in = copy(wg_hbm, wg_v, 1)
        up_in = [copy(wu_hbm, wu_v, 4 + i, pl.ds(lo, hi - lo))
                 for i, (lo, hi) in enumerate(up_spans)]
        down_in = [copy(wd_hbm, wd_v, 4 + len(up_spans) + i, (slice(None), pl.ds(lo, hi - lo)))
                   for i, (lo, hi) in enumerate(early_spans)]
        edge = rows - 2 * _TILE
        split = bands - _TRAILING_BANDS
        trigger_in = [
            copy(wd_hbm, wd_v, 2, (slice(None), pl.ds(early_end, edge - early_end))),
            copy(wd_hbm, wd_v, 2, (pl.ds(0, split), pl.ds(edge, _TILE))),
        ]
        trailing_in = [
            copy(wd_hbm, wd_v, 3, (pl.ds(split, _TRAILING_BANDS), pl.ds(edge, _TILE))),
            copy(wd_hbm, wd_v, 3, (slice(None), pl.ds(edge + _TILE, _TILE))),
        ]
        for cp in router_in + [gate_in] + up_in + down_in + trigger_in + trailing_in:
            cp.start()

        for cp in router_in:
            cp.wait()
        w_r = jnp.broadcast_to(wr_v[...].astype(f32).reshape(1, D), (C, D)).astype(bf16)
        r = jnp.dot(w_r, x_v[...].reshape(D, S), preferred_element_type=f32)
        r = r.astype(bf16).astype(f32)

        token = lax.broadcasted_iota(jnp.int32, (C, S), 1).astype(f32)
        slot = lax.broadcasted_iota(jnp.int32, (C, 1), 0)
        score = jnp.where(r != r, -jnp.inf, r)

        def pick(k, carry):
            free, picked = carry
            best = jnp.max(jnp.where(free < S, score, -jnp.inf), axis=1, keepdims=True)
            who = jnp.min(jnp.where(score == best, free, float(S)), axis=1, keepdims=True)
            return jnp.where(free == who, float(S), free), jnp.where(slot == k, who, picked)

        _, picked = lax.fori_loop(0, C, pick, (token, jnp.zeros((C, 1), f32)))
        routed = token == picked
        r_sel = jnp.sum(jnp.where(routed, r, 0.0), axis=1, keepdims=True)
        weight = jax.nn.sigmoid(r_sel).astype(bf16).astype(f32)
        onehot = routed.astype(f32).astype(bf16)
        x_sel = lax.dot_general(onehot, x_v[...].reshape(D, S), (((1,), (1,)), ((), ())),
                                preferred_element_type=f32).astype(bf16)

        def cols(c):
            return pl.ds(pl.multiple_of(c * _F_CHUNK, _F_CHUNK), _F_CHUNK)

        gate_in.wait()

        @pl.loop(0, F // _F_CHUNK)
        def _(c):
            g = jnp.dot(x_sel, wg_v[:, cols(c)], preferred_element_type=f32)
            g_v[:, cols(c)] = g * jax.nn.sigmoid(g)

        for cp, (lo, hi) in zip(up_in, up_spans):
            cp.wait()

            @pl.loop(0, F // _F_CHUNK)
            def _(c, lo=lo, hi=hi):
                u = jnp.dot(x_sel[:, lo:hi], wu_v[lo:hi, cols(c)], preferred_element_type=f32)
                if lo > 0:
                    u = u + h_v[:, cols(c)]
                if hi == D:
                    u = g_v[:, cols(c)] * u
                h_v[:, cols(c)] = u

        def finish_rows(lo, hi):
            n = bands * (hi - lo)
            y = lax.dot_general(h_v[...].astype(bf16), wd_v[:, lo:hi, :].reshape(n, F),
                                (((1,), (1,)), ((), ())), preferred_element_type=f32)
            y = (y.astype(bf16).astype(f32) * weight).astype(bf16)
            scattered = lax.dot_general(y, onehot, (((0,), (0,)), ((), ())),
                                        preferred_element_type=f32)
            x = x_v[:, lo:hi, :].reshape(n, S).astype(f32)
            out = x + (x * 0.0 + scattered)
            o_v[:, lo:hi, :] = out.astype(bf16).reshape(bands, hi - lo, S)

        for cp, (lo, hi) in zip(down_in, early_spans):
            cp.wait()
            finish_rows(lo, hi)
        for cp in trigger_in:
            cp.wait()
        start_writes(0, early_end)
        finish_rows(early_end, _MID_ROWS)
        start_writes(early_end, _MID_ROWS)
        for cp in trailing_in:
            cp.wait()
        finish_rows(_MID_ROWS, rows)
        start_writes(_MID_ROWS, rows)

    pl.run_scoped(
        read_and_compute,
        pltpu.SemaphoreType.DMA((4 + len(_UP_ROWS) + len(_EARLY_ROWS),)),
    )
    pltpu.make_async_copy(o_v, o_hbm, out_sem).wait()


@jax.jit
def pallas_standalone__moe_arch_mod__prompt_kernel(
    x: jax.Array,
    w_r: jax.Array,
    w_gate: jax.Array,
    w_up: jax.Array,
    w_down: jax.Array,
):
    B, S, D = x.shape
    F = w_gate.shape[1]
    rows = D // _GROUPS
    hbm = pl.BlockSpec(memory_space=pltpu.HBM)
    out_t = pl.pallas_call(
        _mod_kernel,
        in_specs=[hbm] * 5,
        out_specs=hbm,
        out_shape=jax.ShapeDtypeStruct((_GROUPS, rows, S), x.dtype),
        scratch_shapes=[
            pltpu.VMEM((_GROUPS, rows, S), x.dtype),
            pltpu.VMEM((D,), w_r.dtype),
            pltpu.VMEM((D, F), w_gate.dtype),
            pltpu.VMEM((D, F), w_up.dtype),
            pltpu.VMEM((_GROUPS, rows, F), w_down.dtype),
            pltpu.VMEM((_GROUPS, rows, S), x.dtype),
            pltpu.VMEM((_CAPACITY, F), jnp.float32),
            pltpu.VMEM((_CAPACITY, F), jnp.float32),
            pltpu.SemaphoreType.DMA(()),
        ],
        compiler_params=pltpu.CompilerParams(vmem_limit_bytes=64 * 1024 * 1024),
    )(
        x.reshape(S, D).T.reshape(_GROUPS, rows, S),
        w_r,
        w_gate,
        w_up,
        w_down.T.reshape(_GROUPS, rows, F),
    )
    return out_t.reshape(D, S).T.reshape(B, S, D)
```

```python
import jax
import jax.numpy as jnp
from jax import lax
import jax.experimental.pallas as pl
import jax.experimental.pallas.tpu as pltpu

_CAPACITY = 8
_BANDS = 4
_TILE = 8
_LANES = 128
_F_CHUNK = 512

_X_COPY_COLS = 4 * _LANES
_W_COPY_COLS = 6 * _LANES
_QUEUE_DEPTH = 25
_LOOKAHEAD = 52
_TRAILING_COPIES = 10

_EARLY_ROWS = (32, 64, 96)
_MID_ROWS = 128


def _pieces(ref, cols, lo, hi, bands=slice(None)):
    return [
        (bands, pl.ds(r, _TILE), pl.ds(c, cols))
        for r in range(lo, hi, _TILE)
        for c in range(0, ref.shape[-1], cols)
    ]


def _issue_order(copies, spacers):
    high = [(cp, 0) for cp in copies[0::2]]
    low = [(cp, 1) for cp in copies[1::2] + spacers]
    order, low = low[:_QUEUE_DEPTH], low[_QUEUE_DEPTH:]
    for i, entry in enumerate(high):
        order += [entry] + low[i:i + 1]
    return order + low[len(high):]


def _mod_kernel(x_hbm, wr_hbm, wg_hbm, wu_hbm, wd_hbm, o_hbm,
                x_v, wr_v, wg_v, wu_v, wd_v, o_v, g_v, h_v, out_sem):
    bands, rows, S = x_hbm.shape
    D, F = bands * rows, wg_hbm.shape[-1]
    C = _CAPACITY
    f32, bf16 = jnp.float32, jnp.bfloat16

    def start_writes(lo, hi):
        for r in range(lo, hi, _TILE):
            idx = (slice(None), pl.ds(r, _TILE))
            pltpu.make_async_copy(o_v.at[idx], o_hbm.at[idx], out_sem).start()

    def read_and_compute(sems):
        X, WR, GATE, UP, TRIGGER, TRAILING, EARLY = range(7)

        def copy(src, dst, sem, idx=None):
            if idx is not None:
                src, dst = src.at[idx], dst.at[idx]
            return pltpu.make_async_copy(src, dst, sems.at[sem])

        def down_rows(sem, lo, hi):
            return copy(wd_hbm, wd_v, sem, (slice(None), pl.ds(lo, hi - lo)))

        reads = [copy(wr_hbm, wr_v, WR)]
        reads += [copy(x_hbm, x_v, X, i) for i in _pieces(x_hbm, _X_COPY_COLS, 0, rows)]
        end_x = len(reads)
        reads += [copy(wg_hbm, wg_v, GATE, i) for i in _pieces(wg_hbm, _W_COPY_COLS, 0, rows)]
        end_gate = len(reads)
        reads += [copy(wu_hbm, wu_v, UP, i) for i in _pieces(wu_hbm, _W_COPY_COLS, 0, rows)]
        end_up = len(reads)
        early_spans = list(zip((0,) + _EARLY_ROWS[:-1], _EARLY_ROWS))
        end_early = []
        for k, (lo, hi) in enumerate(early_spans):
            reads += [copy(wd_hbm, wd_v, EARLY + k, i)
                      for i in _pieces(wd_hbm, _W_COPY_COLS, lo, hi)]
            end_early.append(len(reads))
        early_end, edge = _EARLY_ROWS[-1], rows - _TILE
        late = (_pieces(wd_hbm, _W_COPY_COLS, early_end, edge)
                + _pieces(wd_hbm, _W_COPY_COLS, edge, rows, pl.ds(0, bands - 1)))
        trigger = [copy(wd_hbm, wd_v, TRIGGER, i) for i in late[:-_TRAILING_COPIES]]
        trailing = [copy(wd_hbm, wd_v, TRAILING, i) for i in late[-_TRAILING_COPIES:]]
        spacers = [copy(wd_hbm, wd_v, TRAILING, i)
                   for i in _pieces(wd_hbm, _LANES, edge, rows, pl.ds(bands - 1, 1))]
        pending = _issue_order(reads + trigger + trailing, spacers)
        total = len(pending)

        def issue_through(position):
            while pending and total - len(pending) < position + _QUEUE_DEPTH + _LOOKAHEAD:
                cp, priority = pending.pop(0)
                cp.start(priority=priority)

        issue_through(end_x)
        copy(wr_hbm, wr_v, WR).wait()
        copy(x_hbm, x_v, X).wait()
        w_r = jnp.broadcast_to(wr_v[...].astype(f32).reshape(1, D), (C, D)).astype(bf16)
        r = jnp.dot(w_r, x_v[...].reshape(D, S), preferred_element_type=f32)
        r = r.astype(bf16).astype(f32)

        token = lax.broadcasted_iota(jnp.int32, (C, S), 1).astype(f32)
        slot = lax.broadcasted_iota(jnp.int32, (C, 1), 0)
        score = jnp.where(r != r, -jnp.inf, r)

        def pick(k, carry):
            free, picked = carry
            best = jnp.max(jnp.where(free < S, score, -jnp.inf), axis=1, keepdims=True)
            who = jnp.min(jnp.where(score == best, free, float(S)), axis=1, keepdims=True)
            return jnp.where(free == who, float(S), free), jnp.where(slot == k, who, picked)

        _, picked = lax.fori_loop(0, C, pick, (token, jnp.zeros((C, 1), f32)))
        routed = token == picked
        r_sel = jnp.sum(jnp.where(routed, r, 0.0), axis=1, keepdims=True)
        weight = jax.nn.sigmoid(r_sel).astype(bf16).astype(f32)
        onehot = routed.astype(f32).astype(bf16)
        issue_through(end_x + (end_gate - end_x) // 3)
        x_sel = lax.dot_general(onehot, x_v[...].reshape(D, S), (((1,), (1,)), ((), ())),
                                preferred_element_type=f32).astype(bf16)

        def cols(c):
            return pl.ds(pl.multiple_of(c * _F_CHUNK, _F_CHUNK), _F_CHUNK)

        issue_through(end_gate)
        copy(wg_hbm, wg_v, GATE).wait()

        @pl.loop(0, F // _F_CHUNK)
        def _(c):
            w = wg_v[:, :, cols(c)].reshape(D, _F_CHUNK)
            g = jnp.dot(x_sel, w, preferred_element_type=f32)
            g_v[:, cols(c)] = g * jax.nn.sigmoid(g)

        issue_through(end_up)
        copy(wu_hbm, wu_v, UP).wait()

        @pl.loop(0, F // _F_CHUNK)
        def _(c):
            w = wu_v[:, :, cols(c)].reshape(D, _F_CHUNK)
            h_v[:, cols(c)] = g_v[:, cols(c)] * jnp.dot(x_sel, w, preferred_element_type=f32)

        def finish_rows(lo, hi):
            n = bands * (hi - lo)
            y = lax.dot_general(h_v[...].astype(bf16), wd_v[:, lo:hi, :].reshape(n, F),
                                (((1,), (1,)), ((), ())), preferred_element_type=f32)
            y = (y.astype(bf16).astype(f32) * weight).astype(bf16)
            scattered = lax.dot_general(y, onehot, (((0,), (0,)), ((), ())),
                                        preferred_element_type=f32)
            x = x_v[:, lo:hi, :].reshape(n, S).astype(f32)
            out = x + (x * 0.0 + scattered)
            o_v[:, lo:hi, :] = out.astype(bf16).reshape(bands, hi - lo, S)

        for k, (lo, hi) in enumerate(early_spans):
            issue_through(end_early[k])
            down_rows(EARLY + k, lo, hi).wait()
            finish_rows(lo, hi)
        issue_through(total)
        for cp in trigger:
            cp.wait()
        start_writes(0, early_end)
        finish_rows(early_end, _MID_ROWS)
        start_writes(early_end, _MID_ROWS)
        for cp in trailing + spacers:
            cp.wait()
        finish_rows(_MID_ROWS, rows)
        start_writes(_MID_ROWS, rows)

    pl.run_scoped(read_and_compute, pltpu.SemaphoreType.DMA((6 + len(_EARLY_ROWS),)))
    pltpu.make_async_copy(o_v, o_hbm, out_sem).wait()


@jax.jit
def pallas_standalone__moe_arch_mod__prompt_kernel(
    x: jax.Array,
    w_r: jax.Array,
    w_gate: jax.Array,
    w_up: jax.Array,
    w_down: jax.Array,
):
    B, S, D = x.shape
    F = w_gate.shape[1]
    rows = D // _BANDS
    hbm = pl.BlockSpec(memory_space=pltpu.HBM)
    out_t = pl.pallas_call(
        _mod_kernel,
        in_specs=[hbm] * 5,
        out_specs=hbm,
        out_shape=jax.ShapeDtypeStruct((_BANDS, rows, S), x.dtype),
        scratch_shapes=[
            pltpu.VMEM((_BANDS, rows, S), x.dtype),
            pltpu.VMEM((D,), w_r.dtype),
            pltpu.VMEM((_BANDS, rows, F), w_gate.dtype),
            pltpu.VMEM((_BANDS, rows, F), w_up.dtype),
            pltpu.VMEM((_BANDS, rows, F), w_down.dtype),
            pltpu.VMEM((_BANDS, rows, S), x.dtype),
            pltpu.VMEM((_CAPACITY, F), jnp.float32),
            pltpu.VMEM((_CAPACITY, F), jnp.float32),
            pltpu.SemaphoreType.DMA(()),
        ],
        compiler_params=pltpu.CompilerParams(vmem_limit_bytes=64 * 1024 * 1024),
    )(
        x.reshape(S, D).T.reshape(_BANDS, rows, S),
        w_r,
        w_gate.reshape(_BANDS, rows, F),
        w_up.reshape(_BANDS, rows, F),
        w_down.T.reshape(_BANDS, rows, F),
    )
    return out_t.reshape(D, S).T.reshape(B, S, D)
```

```python
import jax
import jax.numpy as jnp
from jax import lax
import jax.experimental.pallas as pl
import jax.experimental.pallas.tpu as pltpu

_CAPACITY = 8
_BANDS = 4
_TILE_ROWS, _TILE_COLS = 8, 128
_F_CHUNK = 512

_COPY_COLS = 4 * _TILE_COLS
_QUEUE_DEPTH = 27
_LOOKAHEAD = 52
_TRAILING_COPIES = 14
_SPACERS = 28

_GATE_SPLIT = 40
_UP_SPLIT = 72
_DOWN_STEPS = tuple(((r, r + 16), (r + 64, r + 80)) for r in range(0, 64, 16))
_LAST_ROWS = (128, 144)


def _pieces(lo, hi, col_lo, col_hi, cols=_COPY_COLS, bands=slice(None)):
    return [
        (bands, pl.ds(r, _TILE_ROWS), pl.ds(c, cols))
        for r in range(lo, hi, _TILE_ROWS)
        for c in range(col_lo, col_hi, cols)
    ]


def _issue_order(high, low):
    high, low = [(cp, 0) for cp in high], [(cp, 1) for cp in low]
    order = high[:1] + low[:_QUEUE_DEPTH + 1]
    for i in range(1, len(high)):
        order += [high[i]] + low[_QUEUE_DEPTH + i:_QUEUE_DEPTH + i + 1]
    return order + low[_QUEUE_DEPTH + len(high):]


def _mod_kernel(x_hbm, wr_hbm, wg_hbm, wu_hbm, wd_hbm, o_hbm,
                x_v, wr_v, wg_v, wu_v, wd_v, o_v, g_v, h_v, out_sem):
    bands, rows, S = x_hbm.shape
    D, F = bands * rows, wg_hbm.shape[-1]
    C = _CAPACITY
    f32, bf16 = jnp.float32, jnp.bfloat16

    def start_writes(spans):
        for lo, hi in spans:
            for idx in _pieces(lo, hi, 0, S, cols=S):
                pltpu.make_async_copy(o_v.at[idx], o_hbm.at[idx], out_sem).start()

    def read_and_compute(sems):
        X, WR, GATE, UP, TRIGGER, TRAILING, DOWN = range(7)

        def copy(src, dst, sem, idx=None):
            if idx is not None:
                src, dst = src.at[idx], dst.at[idx]
            return pltpu.make_async_copy(src, dst, sems.at[sem])

        def copies(src, dst, sem, lo, hi):
            return [copy(src, dst, sem, idx) for idx in _pieces(lo, hi, 0, src.shape[-1])]

        low = copies(x_hbm, x_v, X, 0, rows)
        end_x = 2 * len(low)
        low += copies(wg_hbm, wg_v, GATE, 0, _GATE_SPLIT)
        high = copies(wg_hbm, wg_v, GATE, _GATE_SPLIT, rows)
        high.insert(8, copy(wr_hbm, wr_v, WR))
        end_gate = 2 * max(len(low), len(high))
        low += copies(wu_hbm, wu_v, UP, 0, _UP_SPLIT)
        high += copies(wu_hbm, wu_v, UP, _UP_SPLIT, rows)
        end_up = 2 * max(len(low), len(high))
        end_down = []
        for k, (low_rows, high_rows) in enumerate(_DOWN_STEPS):
            low += copies(wd_hbm, wd_v, DOWN + 2 * k, *low_rows)
            high += copies(wd_hbm, wd_v, DOWN + 2 * k + 1, *high_rows)
            end_down.append(2 * max(len(low), len(high)))
        edge, cut = rows - _TILE_ROWS, F - _SPACERS * _TILE_COLS
        late = (_pieces(_LAST_ROWS[0], edge, 0, F) + _pieces(edge, rows, 0, cut)
                + _pieces(edge, rows, cut, F, bands=pl.ds(0, bands - 1)))
        trigger = [copy(wd_hbm, wd_v, TRIGGER, idx) for idx in late[:-_TRAILING_COPIES]]
        trailing = [copy(wd_hbm, wd_v, TRAILING, idx) for idx in late[-_TRAILING_COPIES:]]
        for cp in trigger + trailing:
            (high if len(high) <= len(low) else low).append(cp)
        spacers = [copy(wd_hbm, wd_v, TRAILING, idx)
                   for idx in _pieces(edge, rows, cut, F, _TILE_COLS, pl.ds(bands - 1, 1))]
        pending = _issue_order(high, low + spacers)
        total = len(pending)

        def issue_through(position):
            while pending and total - len(pending) < position + _QUEUE_DEPTH + _LOOKAHEAD:
                cp, priority = pending.pop(0)
                cp.start(priority=priority)

        issue_through(end_x)
        copy(x_hbm, x_v, X).wait()
        copy(wr_hbm, wr_v, WR).wait()
        w_r = jnp.broadcast_to(wr_v[...].astype(f32).reshape(1, D), (C, D)).astype(bf16)
        r = jnp.dot(w_r, x_v[...].reshape(D, S), preferred_element_type=f32)
        r = r.astype(bf16).astype(f32)

        issue_through(end_x + (end_gate - end_x) // 5)
        token = lax.broadcasted_iota(jnp.int32, (C, S), 1).astype(f32)
        slot = lax.broadcasted_iota(jnp.int32, (C, 1), 0)
        score = jnp.where(r != r, -jnp.inf, r)

        def pick(k, carry):
            free, picked = carry
            best = jnp.max(jnp.where(free < S, score, -jnp.inf), axis=1, keepdims=True)
            who = jnp.min(jnp.where(score == best, free, float(S)), axis=1, keepdims=True)
            return jnp.where(free == who, float(S), free), jnp.where(slot == k, who, picked)

        _, picked = lax.fori_loop(0, C, pick, (token, jnp.zeros((C, 1), f32)))
        routed = token == picked
        r_sel = jnp.sum(jnp.where(routed, r, 0.0), axis=1, keepdims=True)
        weight = jax.nn.sigmoid(r_sel).astype(bf16).astype(f32)
        onehot = routed.astype(f32).astype(bf16)
        issue_through(end_x + 3 * (end_gate - end_x) // 5)
        x_sel = lax.dot_general(onehot, x_v[...].reshape(D, S), (((1,), (1,)), ((), ())),
                                preferred_element_type=f32).astype(bf16)

        def project(w_v, step):
            cols = pl.ds(pl.multiple_of(step * _F_CHUNK, _F_CHUNK), _F_CHUNK)
            w = w_v[:, :, cols].reshape(D, _F_CHUNK)
            return cols, jnp.dot(x_sel, w, preferred_element_type=f32)

        def gate_step(step):
            cols, g = project(wg_v, step)
            g_v[:, cols] = g * jax.nn.sigmoid(g)

        def up_step(step):
            cols, u = project(wu_v, step)
            h_v[:, cols] = g_v[:, cols] * u

        steps = F // _F_CHUNK
        for w_hbm, w_v, sem, end, body in ((wg_hbm, wg_v, GATE, end_gate, gate_step),
                                           (wu_hbm, wu_v, UP, end_up, up_step)):
            issue_through(end)
            copy(w_hbm, w_v, sem).wait()
            pl.loop(0, (steps + 1) // 2)(body)
            issue_through(end + _LOOKAHEAD // 2)
            pl.loop((steps + 1) // 2, steps)(body)

        def finish_rows(spans):
            w = jnp.concatenate(
                [wd_v[:, lo:hi, :].reshape(bands * (hi - lo), F) for lo, hi in spans], axis=0)
            y = lax.dot_general(h_v[...].astype(bf16), w, (((1,), (1,)), ((), ())),
                                preferred_element_type=f32)
            y = (y.astype(bf16).astype(f32) * weight).astype(bf16)
            scattered = lax.dot_general(y, onehot, (((0,), (0,)), ((), ())),
                                        preferred_element_type=f32)
            done = 0
            for lo, hi in spans:
                n = bands * (hi - lo)
                x = x_v[:, lo:hi, :].reshape(n, S).astype(f32)
                out = x + (x * 0.0 + scattered[done:done + n])
                o_v[:, lo:hi, :] = out.astype(bf16).reshape(bands, hi - lo, S)
                done += n

        def wait_rows(k):
            issue_through(end_down[k])
            for q, (lo, hi) in enumerate(_DOWN_STEPS[k]):
                copy(wd_hbm, wd_v, DOWN + 2 * k + q, (slice(None), pl.ds(lo, hi - lo))).wait()

        *early_steps, mid_step = _DOWN_STEPS
        for k, spans in enumerate(early_steps):
            wait_rows(k)
            finish_rows(spans)
        issue_through(total)
        wait_rows(len(early_steps))
        for cp in trigger:
            cp.wait()
        start_writes(sorted(span for spans in early_steps for span in spans))
        finish_rows(mid_step)
        start_writes(mid_step)
        for cp in trailing + spacers:
            cp.wait()
        finish_rows([_LAST_ROWS])
        start_writes([_LAST_ROWS])

    pl.run_scoped(read_and_compute, pltpu.SemaphoreType.DMA((6 + 2 * len(_DOWN_STEPS),)))
    pltpu.make_async_copy(o_v, o_hbm, out_sem).wait()


@jax.jit
def pallas_standalone__moe_arch_mod__prompt_kernel(
    x: jax.Array,
    w_r: jax.Array,
    w_gate: jax.Array,
    w_up: jax.Array,
    w_down: jax.Array,
):
    B, S, D = x.shape
    F = w_gate.shape[1]
    rows = D // _BANDS
    assert B == 1 and rows == _LAST_ROWS[1]
    hbm = pl.BlockSpec(memory_space=pltpu.HBM)
    out_t = pl.pallas_call(
        _mod_kernel,
        in_specs=[hbm] * 5,
        out_specs=hbm,
        out_shape=jax.ShapeDtypeStruct((_BANDS, rows, S), x.dtype),
        scratch_shapes=[
            pltpu.VMEM((_BANDS, rows, S), x.dtype),
            pltpu.VMEM((D,), w_r.dtype),
            pltpu.VMEM((_BANDS, rows, F), w_gate.dtype),
            pltpu.VMEM((_BANDS, rows, F), w_up.dtype),
            pltpu.VMEM((_BANDS, rows, F), w_down.dtype),
            pltpu.VMEM((_BANDS, rows, S), x.dtype),
            pltpu.VMEM((_CAPACITY, F), jnp.float32),
            pltpu.VMEM((_CAPACITY, F), jnp.float32),
            pltpu.SemaphoreType.DMA(()),
        ],
        compiler_params=pltpu.CompilerParams(vmem_limit_bytes=64 * 1024 * 1024),
    )(
        x.reshape(S, D).T.reshape(_BANDS, rows, S),
        w_r,
        w_gate.reshape(_BANDS, rows, F),
        w_up.reshape(_BANDS, rows, F),
        w_down.T.reshape(_BANDS, rows, F),
    )
    return out_t.reshape(D, S).T.reshape(B, S, D)
```
